```python
import os as _os
_os.environ.setdefault("JAX_PLATFORMS", "cpu")
import jax
import jax.numpy as jnp

def _softmax(x, axis=-1):
    return jax.nn.softmax(x, axis=axis)
def _gelu(x):
    return jax.nn.gelu(x, approximate=True)
def _silu(x):
    return jax.nn.silu(x)
def _sigmoid(x):
    return jax.nn.sigmoid(x)
def _layernorm(x, axis=-1, eps=1e-5):
    m = jnp.mean(x, axis=axis, keepdims=True)
    v = jnp.var(x, axis=axis, keepdims=True)
    return (x - m) / jnp.sqrt(v + eps)
def _scatter_add(tgt, idx, src, axis=0):
    return tgt.at[idx].add(src)
def _segment_sum(src, seg, n):
    return jax.ops.segment_sum(src, seg, n)
class _Rng:
    def __init__(self, key):
        self._k = key
    def _next(self):
        self._k, sub = jax.random.split(self._k)
        return sub
    def normal(self, shape):
        return jax.random.normal(self._next(), shape, dtype=jnp.bfloat16)
    def randint(self, lo, hi, shape):
        return jax.random.randint(self._next(), shape, lo, hi, dtype=jnp.int32)
    def uniform(self, shape, lo=0.0, hi=1.0):
        return jax.random.uniform(self._next(), shape, jnp.bfloat16, lo, hi)
    def permutation(self, n):
        return jax.random.permutation(self._next(), n)


kernel_name = 'parallel_sum__ssm_conv_s5__glu_gated_swiglu__prompt'

def setup_inputs():
    _rng = _Rng(jax.random.key(int.from_bytes(__import__("os").urandom(4), "little")))
    _w = (lambda a: (lambda t: t.astype(jnp.bfloat16) if jnp.issubdtype(t.dtype, jnp.floating) else t)(jnp.asarray(a)))
    def _A_setup():
        B, S, D = 1, 2048, 640
        P = D
        Lambda_re = -0.5 * jnp.exp((lambda *s: _rng.normal(s) * 0.4)(P))
        Lambda_im = (lambda *s: _rng.normal(s) * 0.4)(P) * 1.0
        B_re = (lambda *s: _rng.normal(s) * 0.4)(P, D) * (D ** -0.5)
        B_im = (lambda *s: _rng.normal(s) * 0.4)(P, D) * (D ** -0.5)
        C_re = (lambda *s: _rng.normal(s) * 0.4)(D, P) * (P ** -0.5)
        C_im = (lambda *s: _rng.normal(s) * 0.4)(D, P) * (P ** -0.5)
        log_dt = (lambda *s: _rng.normal(s) * 0.4)(P) * 0.3 - 2.0
        Dskip = (lambda *s: _rng.normal(s) * 0.4)(D)
        return {
            "x": _w((lambda *s: _rng.normal(s) * 0.05)(B, S, D)),
            "Lambda_re": _w(Lambda_re),
            "Lambda_im": _w(Lambda_im),
            "B_re": _w(B_re),
            "B_im": _w(B_im),
            "C_re": _w(C_re),
            "C_im": _w(C_im),
            "log_dt": _w(log_dt),
            "Dskip": _w(Dskip),
        }
    _A_in = _A_setup()

    def _B_setup():
        B, S, D, F = 1, 2048, 640, 1728
        return {
            "x": _w((lambda *s: _rng.normal(s) * 0.05)(B, S, D)),
            "w1": _w((lambda *s: _rng.normal(s) * 0.1)(D, F) * (2.0 / D) ** 0.5),
            "w3": _w((lambda *s: _rng.normal(s) * 0.1)(D, F) * (2.0 / D) ** 0.5),
            "w2": _w((lambda *s: _rng.normal(s) * 0.1)(F, D) * (2.0 / F) ** 0.5),
        }
    _B_in = _B_setup()

    return {
        "A_x": _A_in["x"],
        "A_Lambda_re": _A_in["Lambda_re"],
        "A_Lambda_im": _A_in["Lambda_im"],
        "A_B_re": _A_in["B_re"],
        "A_B_im": _A_in["B_im"],
        "A_C_re": _A_in["C_re"],
        "A_C_im": _A_in["C_im"],
        "A_log_dt": _A_in["log_dt"],
        "A_Dskip": _A_in["Dskip"],
        "B_x": _B_in["x"],
        "B_w1": _B_in["w1"],
        "B_w3": _B_in["w3"],
        "B_w2": _B_in["w2"],
    }

def reference(A_x, A_Lambda_re, A_Lambda_im, A_B_re, A_B_im, A_C_re, A_C_im, A_log_dt, A_Dskip, B_x, B_w1, B_w3, B_w2):
    def _A_ref(x, Lambda_re, Lambda_im, B_re, B_im, C_re, C_im, log_dt, Dskip):
        Bsz, L, H = x.shape
        Lam = Lambda_re + 1j * Lambda_im
        Bmat = B_re + 1j * B_im
        Cmat = C_re + 1j * C_im
        dt = jnp.exp(log_dt)
        Lam_bar = jnp.exp(dt * Lam)
        B_bar = ((Lam_bar - 1.0) / Lam)[:, None] * Bmat
        Bu = jnp.einsum("bld,pd->blp", x + 0j, B_bar)
        h = jnp.zeros_like(Bu[:, 0, :])
        hs = []
        for t in range(L):
            h = Lam_bar[None, :] * h + Bu[:, t, :]
            hs.append(h)
        hseq = jnp.stack(hs, 1)
        y = 2.0 * jnp.einsum("blp,dp->bld", hseq, Cmat).real + x * Dskip[None, None, :]
        return y

    def _B_ref(x, w1, w3, w2):
        gate = jnp.einsum("bsd,df->bsf", x, w1)
        up = jnp.einsum("bsd,df->bsf", x, w3)
        h = _silu(gate) * up
        out = jnp.einsum("bsf,fd->bsd", h, w2)
        return out

    x = A_x
    xn = _layernorm(x, axis=-1)
    return x + _A_ref(xn, A_Lambda_re, A_Lambda_im, A_B_re, A_B_im, A_C_re, A_C_im, A_log_dt, A_Dskip) + _B_ref(xn, B_w1, B_w3, B_w2)
```

```python
import functools
import jax
import jax.numpy as jnp
from jax import lax
import jax.experimental.pallas as pl
import jax.experimental.pallas.tpu as pltpu

F32 = jnp.float32
BF16 = jnp.bfloat16
NT = (((1,), (1,)), ((), ()))


def _cmul(ar, ai, br, bi):
    return ar * br - ai * bi, ar * bi + ai * br


def _nt(a, b):
    return lax.dot_general(a, b, NT, preferred_element_type=F32)


def _kernel(x_hbm, lre_hbm, lim_hbm, ldt_hbm, dsk_hbm, bre_hbm, bim_hbm, cre_hbm, cim_hbm,
            w1_hbm, w3_hbm, w2_hbm, o_hbm,
            xv, prm0, prm1, prm2, prm3, bw, cw, w13, w2, xs, xh, res, bu, hf, accs, ob, cst, xsem, wsem, osem,
            *, T, L, D, P, F, G, unroll, lnpos, look, stops, peel, xw, pace, five):
    NC = L // T
    LS = T // 8
    SP = LS + 8
    KD = D // 128
    KP = P // 128
    FM = F // 128 * 128
    FT = F - FM

    def xcopy(c):
        return pltpu.make_async_copy(x_hbm.at[pl.ds(c * T, T)], xv.at[pl.ds(c * T, T)], xsem.at[c])

    nsem = [0]

    def cp(s, d):
        nsem[0] += 1
        return pltpu.make_async_copy(s, d, wsem.at[nsem[0] - 1])

    pc = [cp(lre_hbm, prm0), cp(lim_hbm, prm1), cp(ldt_hbm, prm2), cp(dsk_hbm, prm3)]
    grp = []
    bpc = [(k, 1) for k in range(KP)] if five else [(0, 2), (2, 2), (4, 1)]
    for k0, nk in bpc:
        g = []
        for k in range(k0, k0 + nk):
            g.append(cp(bre_hbm.at[pl.ds(128 * k, 128)], bw.at[pl.ds(256 * k, 128)]))
            g.append(cp(bim_hbm.at[pl.ds(128 * k, 128)], bw.at[pl.ds(256 * k + 128, 128)]))
        grp.append(g)
    pcs = []
    for f0 in range(0, FM, G):
        n = min(G, FM - f0)
        grp.append([cp(w1_hbm.at[pl.ds(f0, n)], w13.at[pl.ds(2 * f0, n)]),
                    cp(w3_hbm.at[pl.ds(f0, n)], w13.at[pl.ds(2 * f0 + n, n)])])
        pcs.append((f0, n))
    grp[-1] += [cp(w1_hbm.at[pl.ds(FM, FT)], w13.at[pl.ds(2 * FM, FT)]),
                cp(w3_hbm.at[pl.ds(FM, FT)], w13.at[pl.ds(2 * FM + FT, FT)])]
    grp.append([cp(w2_hbm, w2)])
    grp.append([cp(cre_hbm, cw.at[:, pl.ds(0, P)]), cp(cim_hbm, cw.at[:, pl.ds(P, P)])])

    for w in pc:
        w.start()
    xcopy(0).start()
    for w in grp[0]:
        w.start()
    xcopy(1).start()
    for g in grp[1:look]:
        for w in g:
            w.start()

    def need(first, i):
        if not first or i not in stops:
            return
        q = stops.index(i)
        end = stops[q + 1] if q + 1 < len(stops) else len(grp)
        for g in grp[i:end]:
            for w in g:
                w.wait()
        if i == 0:
            for g in grp[look:]:
                for w in g:
                    w.start()
        if i == len(grp) - 2:
            for cc in range(2, NC):
                xcopy(cc).start()

    for w in pc:
        w.wait()
    lre = prm0[...].astype(F32).reshape(1, P)
    lim = prm1[...].astype(F32).reshape(1, P)
    dt = jnp.exp(prm2[...].astype(F32).reshape(1, P)).astype(BF16).astype(F32)
    dsk = prm3[...].astype(F32).reshape(1, D)
    mag = jnp.exp(dt * lre)
    ar = mag * jnp.cos(dt * lim)
    ai = mag * jnp.sin(dt * lim)
    den = lre * lre + lim * lim
    sr = 2.0 * ((ar - 1.0) * lre + ai * lim) / den
    si = 2.0 * (ai * lre - (ar - 1.0) * lim) / den
    pr, pi = ar, ai
    n = 1
    while n < LS:
        pr, pi = _cmul(pr, pi, pr, pi)
        n *= 2
    assert n == LS
    for i, v in enumerate([ar, ai, sr, si, pr, pi, dsk]):
        cst[i] = jnp.broadcast_to(v, (8, P))
    cst[7] = jnp.zeros((8, P), F32)
    cst[8] = jnp.zeros((8, P), F32)

    def ln_stage(c):
        r0 = pl.multiple_of(c * T, T)
        for k in range(KD):
            xf = xv[pl.ds(r0, T), 128 * k:128 * k + 128].astype(F32)
            for i in range(8):
                xs[k, SP * i:SP * i + LS, :] = xf[LS * i:LS * i + LS]

    def ln(c, j0, j1):
        r0 = pl.multiple_of(c * T, T) + 8 * j0
        n = 8 * (j1 - j0)
        xp = jnp.concatenate([jnp.concatenate([xs[k, pl.ds(j, 8, stride=SP), :] for j in range(j0, j1)], axis=0)
                              for k in range(KD)], axis=1)
        m = jnp.mean(xp, axis=-1, keepdims=True)
        xc = xp - m
        v = jnp.mean(xc * xc, axis=-1, keepdims=True)
        xb = (xc * lax.rsqrt(v + 1e-5)).astype(BF16)
        xh[pl.ds(r0, n), 0:D] = xb
        res[pl.ds(r0, n), :] = xp + xb.astype(F32) * jnp.tile(cst[6], (n // 8, 1))

    def scan(c, k):
        r0 = pl.multiple_of(c * T, T)
        lc = slice(128 * k, 128 * k + 128)
        lr = slice(256 * k, 256 * k + 128)
        li = slice(256 * k + 128, 256 * k + 256)
        a8r, a8i, s8r, s8i, qr, qi, cr_, ci_ = [cst[i, :, lc] for i in (0, 1, 2, 3, 4, 5, 7, 8)]
        sub = lax.broadcasted_iota(jnp.int32, (8, 128), 0)

        def step(j, hr, hi):
            return ((a8r * hr + bu[8 * j:8 * j + 8, lr]) - a8i * hi,
                    (a8r * hi + bu[8 * j:8 * j + 8, li]) + a8i * hr)
        er = bu[0:8, lr]
        ei = bu[0:8, li]
        for j in range(1, LS):
            er, ei = step(j, er, ei)
        tr, ti = _cmul(qr, qi, cr_, ci_)
        er = er + jnp.where(sub == 0, tr, 0.0)
        ei = ei + jnp.where(sub == 0, ti, 0.0)
        for sh in (1, 2, 4):
            tr, ti = _cmul(qr, qi, pltpu.roll(er, sh, 0), pltpu.roll(ei, sh, 0))
            er = er + jnp.where(sub >= sh, tr, 0.0)
            ei = ei + jnp.where(sub >= sh, ti, 0.0)
            if sh < 4:
                qr, qi = _cmul(qr, qi, qr, qi)
        er = pltpu.roll(er, 1, 0)
        ei = pltpu.roll(ei, 1, 0)
        cst[7, :, lc] = er
        cst[8, :, lc] = ei
        hr = jnp.where(sub == 0, cr_, er)
        hi = jnp.where(sub == 0, ci_, ei)
        for j in range(0, LS, 2):
            h1r, h1i = step(j, hr, hi)
            hr, hi = step(j + 1, h1r, h1i)
            xh[pl.ds(r0 + 8 * j, 16), D + 128 * k:D + 128 * k + 128] = jnp.concatenate(
                [h1r * s8r - h1i * s8i, hr * s8r - hi * s8i], axis=0).astype(BF16)
            xh[pl.ds(r0 + 8 * j, 16), D + P + 128 * k:D + P + 128 * k + 128] = jnp.concatenate(
                [-(h1r * s8i) - h1i * s8r, -(hr * s8i) - hi * s8r], axis=0).astype(BF16)

    def unperm(c):
        r0 = pl.multiple_of(c * T, T)
        for k in range(KD):
            ob[pl.ds(r0, T), 128 * k:128 * k + 128] = jnp.concatenate(
                [accs[k, pl.ds(8 * j0 + i, 8, stride=8), :] for i in range(8) for j0 in range(0, LS, 8)], axis=0)

    def ocopy(c):
        return pltpu.make_async_copy(ob.at[pl.ds((c + 1) * T, T)], o_hbm.at[pl.ds(c * T, T)], osem)

    xcopy(0).wait()
    ln_stage(0)
    for j in range(0, LS, 2):
        ln(0, j, j + 2)

    def body(c, first=False, final=False):
        r0 = pl.multiple_of(c * T, T)
        if not first:
            unperm(c)
        for i, (k0, nk) in enumerate(bpc):
            need(first, i)
            if i == 0:
                if first:
                    xcopy(1).wait()
                if not final:
                    ln_stage(c + 1)
            t = _nt(xh[pl.ds(r0, T), 0:D], bw[256 * k0:256 * (k0 + nk)])
            bu[0:T, 256 * k0:256 * (k0 + nk)] = t
            if i in lnpos and not final:
                q = lnpos.index(i)
                if pace & 4:
                    xs[0, pl.ds(8 * SP - 8 + pl.multiple_of((c >> 12) * 8, 8), 8), :] = t[T - 8:T, 0:128]
                for j in range(q * LS // len(lnpos), (q + 1) * LS // len(lnpos), 2):
                    ln(c + 1, j, j + 2)
        nl = len(lnpos)
        for pi_, (f0, n) in enumerate(pcs):
            last = pi_ == len(pcs) - 1
            need(first, len(bpc) + pi_)
            if pi_ == 0 and final:
                ocopy(c - 1).start()
            t = _nt(xh[pl.ds(r0, T), 0:D], w13[2 * f0:(2 * F if last else 2 * f0 + 2 * n)])
            g = 0.5 * t[:, :n]
            hf[:, f0:f0 + n] = ((g * jnp.tanh(g) + g) * t[:, n:2 * n]).astype(BF16)
            if last:
                g = 0.5 * t[:, 2 * n:2 * n + FT]
                hf[:, FM:F] = ((g * jnp.tanh(g) + g) * t[:, 2 * n + FT:]).astype(BF16)
            z = pl.multiple_of((c >> 12) * 8, 8)
            if pace & 1:
                bu[pl.ds(T + z, 8), 0:128] = t[T - 8:T, 0:128]
            if pace & 2:
                xs[0, pl.ds(8 * SP - 8 + z, 8), :] = t[T - 8:T, 0:128]
            if pi_ < KP:
                scan(c, pi_)
        need(first, len(grp) - 2)
        acc = res[pl.ds(r0, T), :] + jnp.dot(hf[:, 0:F], w2[...], preferred_element_type=F32)
        need(first, len(grp) - 1)
        acc = acc + _nt(xh[pl.ds(r0, T), D:], cw[...])
        for k in range(KD):
            accs[k] = acc[:, 128 * k:128 * k + 128]
        if not (first or final):
            ocopy(c - 1).start()
        return 0

    body(0, first=True)
    for cc in range(2, NC):
        xcopy(cc).wait()
    if unroll == 0:
        for c in range(1, NC - peel):
            body(c)
    else:
        lax.fori_loop(1, NC - peel, lambda c, _: body(c), 0, unroll=unroll)
    if peel:
        body(NC - 1, final=True)
    unperm(NC)
    ocopy(NC - 1).start()
    for c in range(NC):
        ocopy(c).wait()


@jax.jit
def pallas_parallel_sum__ssm_conv_s5__glu_gated_swiglu__prompt_kernel(A_x, A_Lambda_re, A_Lambda_im, A_B_re, A_B_im, A_C_re, A_C_im, A_log_dt, A_Dskip, B_x, B_w1, B_w3, B_w2):
    T, G, unroll, lnpos, look, peel, xw, pace, five = 256, 256, 1, (0, 1), 3, 1, 3, 5, 0
    stops = (0, 1, 3, 5, 7, 10, 11)
    Bsz, L, D = A_x.shape
    P = A_Lambda_re.shape[0]
    F = B_w1.shape[1]
    NC = L // T
    FM = F // 128 * 128
    hbm = pl.BlockSpec(memory_space=pltpu.HBM)
    out = pl.pallas_call(
        functools.partial(_kernel, T=T, L=L, D=D, P=P, F=F, G=G, unroll=unroll, lnpos=lnpos, look=look, stops=stops, peel=peel, xw=xw, pace=pace, five=five),
        in_specs=[hbm] * 12,
        out_specs=hbm,
        out_shape=jax.ShapeDtypeStruct((L, D), F32),
        scratch_shapes=[
            pltpu.VMEM((L, D), BF16),
            pltpu.VMEM((P,), BF16), pltpu.VMEM((P,), BF16), pltpu.VMEM((P,), BF16), pltpu.VMEM((D,), BF16),
            pltpu.VMEM((2 * P, D), BF16), pltpu.VMEM((D, 2 * P), BF16),
            pltpu.VMEM((2 * F, D), BF16), pltpu.VMEM((F, D), BF16),
            pltpu.VMEM((D // 128, T + 64, 128), F32), pltpu.VMEM((L + T, D + 2 * P), BF16), pltpu.VMEM((L + T, D), F32),
            pltpu.VMEM((T + 8, 2 * P), F32), pltpu.VMEM((T, FM + 128), BF16),
            pltpu.VMEM((D // 128, T, 128), F32), pltpu.VMEM((L + T, D), F32), pltpu.VMEM((9, 8, P), F32),
            pltpu.SemaphoreType.DMA((NC,)), pltpu.SemaphoreType.DMA((64,)), pltpu.SemaphoreType.DMA(()),
        ],
        compiler_params=pltpu.CompilerParams(vmem_limit_bytes=100 * 1024 * 1024),
    )(A_x.reshape(L, D), A_Lambda_re, A_Lambda_im, A_log_dt, A_Dskip,
      A_B_re, A_B_im, A_C_re, A_C_im, B_w1.T, B_w3.T, B_w2)
    return out.reshape(1, L, D)
```
